```python
import jax
import jax.numpy as jnp

def _softmax(x, axis=-1):
    return jax.nn.softmax(x, axis=axis)
def _gelu(x):
    return jax.nn.gelu(x, approximate=True)
def _silu(x):
    return jax.nn.silu(x)
def _sigmoid(x):
    return jax.nn.sigmoid(x)
def _layernorm(x, axis=-1, eps=1e-5):
    m = jnp.mean(x, axis=axis, keepdims=True)
    v = jnp.var(x, axis=axis, keepdims=True)
    return (x - m) / jnp.sqrt(v + eps)
def _scatter_add(tgt, idx, src, axis=0):
    return tgt.at[idx].add(src)
def _segment_sum(src, seg, n):
    return jax.ops.segment_sum(src, seg, n)
class _Rng:
    def __init__(self, key):
        self._k = key
    def _next(self):
        self._k, sub = jax.random.split(self._k)
        return sub
    def normal(self, shape):
        return jax.random.normal(self._next(), shape, dtype=jnp.bfloat16)
    def randint(self, lo, hi, shape):
        return jax.random.randint(self._next(), shape, lo, hi, dtype=jnp.int32)
    def uniform(self, shape, lo=0.0, hi=1.0):
        return jax.random.uniform(self._next(), shape, jnp.bfloat16, lo, hi)
    def permutation(self, n):
        return jax.random.permutation(self._next(), n)


kernel_name = 'parallel_sum__sliding_block_cached__mixer_s_mlp__decode'

def setup_inputs():
    _rng = _Rng(jax.random.key(int.from_bytes(__import__("os").urandom(4), "little")))
    _w = (lambda a: (lambda t: t.astype(jnp.bfloat16) if jnp.issubdtype(t.dtype, jnp.floating) else t)(jnp.asarray(a)))
    def _A_setup():
        B, Sq, D = 4, 1, 512
        Hq, Hkv, Sk, Dh = 32, 32, 8192, 128
        assert Hq % Hkv == 0, (Hq, Hkv)
        return {
            "x": _w((lambda *s: _rng.normal(s) * 0.05)(B, Sq, D)),
            "k_cache": _w((lambda *s: _rng.normal(s) * 0.05)(B, Hkv, Sk, Dh)),
            "v_cache": _w((lambda *s: _rng.normal(s) * 0.05)(B, Hkv, Sk, Dh)),
            "wq": _w((lambda *s: _rng.normal(s) * 0.05)(D, Hq * Dh) * (D ** -0.5)),
            "wo": _w((lambda *s: _rng.normal(s) * 0.05)(Hq * Dh, D) * ((Hq * Dh) ** -0.5)),
        }
    _A_in = _A_setup()

    def _B_setup():
        B, S, D, F = 4, 1, 512, 1376
        return {
            "x":  _w((lambda *s: _rng.normal(s) * 0.05)(B, S, D)),
            "w1": _w((lambda *s: _rng.normal(s) * 0.05)(D, D) * (D ** -0.5)),
            "w2": _w((lambda *s: _rng.normal(s) * 0.05)(D, D) * (D ** -0.5)),
            "w3": _w((lambda *s: _rng.normal(s) * 0.05)(D, F) * (D ** -0.5)),
            "w4": _w((lambda *s: _rng.normal(s) * 0.05)(F, D) * (F ** -0.5)),
        }
    _B_in = _B_setup()

    return {
        "A_x": _A_in["x"],
        "A_k_cache": _A_in["k_cache"],
        "A_v_cache": _A_in["v_cache"],
        "A_wq": _A_in["wq"],
        "A_wo": _A_in["wo"],
        "B_x": _B_in["x"],
        "B_w1": _B_in["w1"],
        "B_w2": _B_in["w2"],
        "B_w3": _B_in["w3"],
        "B_w4": _B_in["w4"],
    }

def reference(A_x, A_k_cache, A_v_cache, A_wq, A_wo, B_x, B_w1, B_w2, B_w3, B_w4):
    def _A_ref(x, k_cache, v_cache, wq, wo):
        B, Sq, D = x.shape
        Hq, Dh = 32, 128
        Hkv, Sk = k_cache.shape[1], k_cache.shape[2]
        W = min(4096, max(256, Sk // 4))
        rep = Hq // Hkv
        q = (lambda x, *d: x.transpose(*d))((x @ wq).reshape(B, Sq, Hq, Dh), 0, 2, 1, 3)
        k = jnp.repeat(k_cache[:, :, Sk - W:, :], rep, axis=1)
        v = jnp.repeat(v_cache[:, :, Sk - W:, :], rep, axis=1)
        scores = jnp.einsum("bhqd,bhkd->bhqk", q, k) * (Dh ** -0.5)
        p = _softmax(scores, axis=-1)
        o = jnp.einsum("bhqk,bhkd->bhqd", p, v)
        return (lambda x, *d: x.transpose(*d))(o, 0, 2, 1, 3).reshape(B, Sq, Hq * Dh) @ wo

    def _B_ref(x, w1, w2, w3, w4):
        B, S, D = x.shape
        h = _gelu(_layernorm(x, axis=-1) @ w1)
        c = D // 4
        g0 = jnp.pad(h[:, :, 0*c:1*c], ((0, 0), (1, 0), (0, 0)))[:, :S, :]
        g1 = jnp.pad(h[:, :, 1*c:2*c], ((0, 0), (0, 1), (0, 0)))[:, 1:, :]
        g2 = jnp.pad(h[:, :, 2*c:3*c], ((0, 0), (2, 0), (0, 0)))[:, :S, :]
        g3 = jnp.pad(h[:, :, 3*c:   ], ((0, 0), (0, 2), (0, 0)))[:, 2:, :]
        hs = jnp.concatenate([g0, g1, g2, g3], axis=-1) @ w2
        x1 = x + hs
        h2 = _gelu(_layernorm(x1, axis=-1) @ w3) @ w4
        return x1 + h2

    x = A_x
    xn = _layernorm(x, axis=-1)
    return x + _A_ref(xn, A_k_cache, A_v_cache, A_wq, A_wo) + _B_ref(xn, B_w1, B_w2, B_w3, B_w4)
```

```python
import functools

import jax
import jax.numpy as jnp
from jax import lax
import jax.experimental.pallas as pl
import jax.experimental.pallas.tpu as pltpu

_HQ = 32
_DH = 128
_EPS = 1e-5
_ROWS = 8
_NT = (((1,), (1,)), ((), ()))


def _layernorm(x):
    m = jnp.mean(x, axis=-1, keepdims=True)
    c = x - m
    v = jnp.mean(c * c, axis=-1, keepdims=True)
    return c / jnp.sqrt(v + _EPS)


def _kernel(x_hbm, k_hbm, v_hbm, wq_hbm, wo_hbm, w3t_hbm, w4_hbm, out_ref,
            x_buf, wq_buf, wo_buf, w3_buf, w4_buf, k_buf, v_buf, q_scr, o_scr,
            w_sem, wo_sem, k_sem, v_sem, *, window, nbuf, wo_pieces):
    batch, heads, sk, dh = k_hbm.shape
    f32, bf16 = jnp.float32, jnp.bfloat16

    def k_copy(h, slot):
        return pltpu.make_async_copy(
            k_hbm.at[:, h, pl.ds(sk - window, window), :], k_buf.at[slot], k_sem.at[slot])

    def v_copy(h, slot):
        return pltpu.make_async_copy(
            v_hbm.at[:, h, pl.ds(sk - window, window), :], v_buf.at[slot], v_sem.at[slot])

    def wo_copy(i):
        h0, nh = wo_pieces[i]
        rows = pl.ds(h0 * dh, nh * dh)
        return pltpu.make_async_copy(wo_hbm.at[rows, :], wo_buf.at[rows, :], wo_sem.at[i])

    x_copy = pltpu.make_async_copy(x_hbm, x_buf, w_sem.at[0])
    wq_copy = pltpu.make_async_copy(wq_hbm, wq_buf, w_sem.at[1])
    w3_copy = pltpu.make_async_copy(w3t_hbm, w3_buf, w_sem.at[2])
    w4_copy = pltpu.make_async_copy(w4_hbm, w4_buf, w_sem.at[3])

    wq_copy.start()
    x_copy.start()
    for i in range(nbuf):
        k_copy(i, i).start()
        v_copy(i, i).start()

    x_copy.wait()
    x = x_buf[...].astype(f32)
    xn = _layernorm(x)
    ln2 = _layernorm(xn)
    pad = jnp.zeros((_ROWS - batch, x.shape[1]), f32)
    xn_p = jnp.concatenate([xn, pad], axis=0).astype(bf16)
    ln2_p = jnp.concatenate([ln2, pad], axis=0).astype(bf16)
    resid = x + xn

    wq_copy.wait()
    q = jnp.dot(xn_p, wq_buf[...], preferred_element_type=f32)
    for h in range(heads):
        q_scr[h] = q[:, h * dh:(h + 1) * dh]

    scale = dh ** -0.5
    row_s = lax.broadcasted_iota(jnp.int32, (_ROWS, window), 0)
    row_o = lax.broadcasted_iota(jnp.int32, (_ROWS, dh), 0)

    def head(h, _):
        slot = lax.rem(h, nbuf)
        qh = q_scr[h].astype(bf16)

        k_copy(h, slot).wait()
        s = None
        for b in range(batch):
            sb = lax.dot_general(qh, k_buf[slot, b], _NT, preferred_element_type=f32)
            s = sb if s is None else jnp.where(row_s == b, sb, s)

        @pl.when(h + nbuf < heads)
        def _():
            k_copy(h + nbuf, slot).start()

        s = s * scale
        m = jnp.max(s, axis=-1, keepdims=True)
        p = jnp.exp(s - m)
        l = jnp.sum(p, axis=-1, keepdims=True)
        p = p.astype(bf16)

        v_copy(h, slot).wait()
        o = None
        for b in range(batch):
            ob = jnp.dot(p, v_buf[slot, b], preferred_element_type=f32)
            o = ob if o is None else jnp.where(row_o == b, ob, o)
        o_scr[h] = o / l

        @pl.when(h + nbuf < heads)
        def _():
            v_copy(h + nbuf, slot).start()

        @pl.when(h + nbuf == heads - 1)
        def _():
            w3_copy.start()
            w4_copy.start()
            for i in range(len(wo_pieces)):
                wo_copy(i).start()

    lax.fori_loop(0, heads, head, None)

    w3_copy.wait()
    hid = lax.dot_general(ln2_p, w3_buf[...], _NT, preferred_element_type=f32)
    hid = jax.nn.gelu(hid, approximate=True).astype(bf16)
    w4_copy.wait()
    acc = jnp.dot(hid, w4_buf[...], preferred_element_type=f32)

    for i, (h0, nh) in enumerate(wo_pieces):
        o = jnp.concatenate([o_scr[h] for h in range(h0, h0 + nh)], axis=1).astype(bf16)
        wo_copy(i).wait()
        acc = acc + jnp.dot(o, wo_buf[pl.ds(h0 * dh, nh * dh), :], preferred_element_type=f32)

    out_ref[...] = (resid + acc[:batch]).astype(out_ref.dtype)


def _pieces(sizes):
    out, h0 = [], 0
    for n in sizes:
        out.append((h0, n))
        h0 += n
    return tuple(out)


def _build(A_x, A_k_cache, A_v_cache, A_wq, A_wo, B_w3, B_w4, *, nbuf=4,
           wo_sizes=(8, 8, 8, 4, 2, 1, 1)):
    batch, sq, d = A_x.shape
    _, heads, sk, dh = A_k_cache.shape
    assert sq == 1 and heads == _HQ and dh == _DH and batch <= _ROWS
    assert sum(wo_sizes) == heads
    window = min(4096, max(256, sk // 4))
    ff = B_w3.shape[1]
    wo_pieces = _pieces(wo_sizes)
    dt = A_x.dtype

    hbm = pl.BlockSpec(memory_space=pl.ANY)
    out = pl.pallas_call(
        functools.partial(_kernel, window=window, nbuf=nbuf, wo_pieces=wo_pieces),
        out_shape=jax.ShapeDtypeStruct((batch, d), dt),
        in_specs=[hbm] * 7,
        out_specs=pl.BlockSpec((batch, d), lambda: (0, 0)),
        scratch_shapes=[
            pltpu.VMEM((batch, d), dt),
            pltpu.VMEM(A_wq.shape, A_wq.dtype),
            pltpu.VMEM(A_wo.shape, A_wo.dtype),
            pltpu.VMEM((ff, d), B_w3.dtype),
            pltpu.VMEM((ff, d), B_w4.dtype),
            pltpu.VMEM((nbuf, batch, window, dh), A_k_cache.dtype),
            pltpu.VMEM((nbuf, batch, window, dh), A_v_cache.dtype),
            pltpu.VMEM((heads, _ROWS, dh), jnp.float32),
            pltpu.VMEM((heads, _ROWS, dh), jnp.float32),
            pltpu.SemaphoreType.DMA((4,)),
            pltpu.SemaphoreType.DMA((len(wo_pieces),)),
            pltpu.SemaphoreType.DMA((nbuf,)),
            pltpu.SemaphoreType.DMA((nbuf,)),
        ],
        compiler_params=pltpu.CompilerParams(vmem_limit_bytes=100 * 2**20),
    )(A_x.reshape(batch, d), A_k_cache, A_v_cache, A_wq, A_wo, B_w3.T, B_w4)
    return out.reshape(batch, sq, d)


@jax.jit
def pallas_parallel_sum__sliding_block_cached__mixer_s_mlp__decode_kernel(
    A_x: jax.Array,
    A_k_cache: jax.Array,
    A_v_cache: jax.Array,
    A_wq: jax.Array,
    A_wo: jax.Array,
    B_x: jax.Array,
    B_w1: jax.Array,
    B_w2: jax.Array,
    B_w3: jax.Array,
    B_w4: jax.Array,
):
    return _build(A_x, A_k_cache, A_v_cache, A_wq, A_wo, B_w3, B_w4)
```

```python
import functools

import jax
import jax.numpy as jnp
from jax import lax
import jax.experimental.pallas as pl
import jax.experimental.pallas.tpu as pltpu

_HEADS = 32
_HEAD_DIM = 128
_EPS = 1e-5
_ROWS = 8
_SLOTS = 2
_WO_HEADS = (23, 6, 2, 1)
_NT = (((1,), (1,)), ((), ()))


def _layernorm(x):
    m = jnp.mean(x, axis=-1, keepdims=True)
    c = x - m
    v = jnp.mean(c * c, axis=-1, keepdims=True)
    return c / jnp.sqrt(v + _EPS)


def _compute(x_hbm, k_hbm, v_hbm, wq_hbm, wo_hbm, w3t_hbm, w4_hbm,
             x_buf, wq_buf, wo_buf, w3t_buf, w4_buf, k_buf, v_buf, o_buf, sems):
    batch, heads, sk, dh = k_hbm.shape
    window = k_buf.shape[2]
    f32, mxu_dtype = jnp.float32, k_buf.dtype
    keys = pl.ds(sk - window, window)
    wo_rows = [pl.ds(sum(_WO_HEADS[:i]) * dh, n * dh) for i, n in enumerate(_WO_HEADS)]

    def k_copy(h, slot):
        return pltpu.make_async_copy(k_hbm.at[:, h, keys, :], k_buf.at[slot], sems.at[2 * slot])

    def v_copy(h, slot):
        return pltpu.make_async_copy(v_hbm.at[:, h, keys, :], v_buf.at[slot], sems.at[2 * slot + 1])

    def wo_copy(i):
        return pltpu.make_async_copy(wo_hbm.at[wo_rows[i], :], wo_buf.at[wo_rows[i], :], sems.at[i])

    def start_stream(w_sem):
        copies = [
            pltpu.make_async_copy(src, dst, w_sem)
            for src, dst in ((wq_hbm, wq_buf), (x_hbm, x_buf), (w3t_hbm, w3t_buf), (w4_hbm, w4_buf))
        ]
        for c in copies:
            c.start()

        def prime(i, _):
            k_copy(i, i).start()
            v_copy(i, i).start()

        lax.fori_loop(0, _SLOTS, prime, None)
        for c in copies:
            c.wait()

    pl.run_scoped(start_stream, pltpu.SemaphoreType.DMA)

    x = x_buf[...].astype(f32)
    xn = _layernorm(x)
    filler = jnp.zeros((_ROWS - batch, x.shape[1]), f32)

    def padded(a):
        return jnp.concatenate([a, filler], axis=0)

    xn_lhs = padded(xn).astype(mxu_dtype)
    hid = lax.dot_general(padded(_layernorm(xn)).astype(mxu_dtype), w3t_buf[...], _NT,
                          preferred_element_type=f32)
    hid = jax.nn.gelu(hid, approximate=True).astype(mxu_dtype)
    acc = padded(x + xn) + jnp.dot(hid, w4_buf[...], preferred_element_type=f32)

    s_row = lax.broadcasted_iota(jnp.int32, (_ROWS, window), 0)
    o_row = lax.broadcasted_iota(jnp.int32, (_ROWS, dh), 0)

    def head(h, _):
        slot = lax.rem(h, _SLOTS)
        cols = pl.ds(pl.multiple_of(h * dh, dh), dh)

        def refill(copy, first_piece):
            pl.when(h + _SLOTS < heads)(lambda: copy(h + _SLOTS, slot).start())
            for j in range(_SLOTS):
                pl.when(h == heads - _SLOTS + j)(wo_copy(2 * j + first_piece).start)

        q = jnp.dot(xn_lhs, wq_buf[:, cols], preferred_element_type=f32).astype(mxu_dtype)

        k_copy(h, slot).wait()
        s = lax.dot_general(q, k_buf[slot, 0], _NT, preferred_element_type=f32)
        for b in range(1, batch):
            s_b = lax.dot_general(q, k_buf[slot, b], _NT, preferred_element_type=f32)
            s = jnp.where(s_row == b, s_b, s)
        refill(k_copy, 0)

        s = s * (dh ** -0.5)
        p = jnp.exp(s - jnp.max(s, axis=-1, keepdims=True))
        denom = jnp.sum(p, axis=-1, keepdims=True)
        p = p.astype(mxu_dtype)

        v_copy(h, slot).wait()
        o = jnp.dot(p, v_buf[slot, 0], preferred_element_type=f32)
        for b in range(1, batch):
            o_b = jnp.dot(p, v_buf[slot, b], preferred_element_type=f32)
            o = jnp.where(o_row == b, o_b, o)
        o_buf[:, cols] = o / denom
        refill(v_copy, 1)

    lax.fori_loop(0, heads, head, None)

    for i, rows in enumerate(wo_rows):
        o = o_buf[:, rows].astype(mxu_dtype)
        wo_copy(i).wait()
        acc = acc + jnp.dot(o, wo_buf[rows, :], preferred_element_type=f32)
    return acc


def _kernel(x_hbm, k_hbm, v_hbm, wq_hbm, wo_hbm, w3t_hbm, w4_hbm, out_ref, *buffers):
    acc = pl.run_scoped(
        functools.partial(_compute, x_hbm, k_hbm, v_hbm, wq_hbm, wo_hbm, w3t_hbm, w4_hbm, *buffers),
        pltpu.SemaphoreType.DMA((2 * _SLOTS,)),
    )
    out_ref[...] = acc[:out_ref.shape[0]].astype(out_ref.dtype)


@jax.jit
def pallas_parallel_sum__sliding_block_cached__mixer_s_mlp__decode_kernel(
    A_x: jax.Array,
    A_k_cache: jax.Array,
    A_v_cache: jax.Array,
    A_wq: jax.Array,
    A_wo: jax.Array,
    B_x: jax.Array,
    B_w1: jax.Array,
    B_w2: jax.Array,
    B_w3: jax.Array,
    B_w4: jax.Array,
):
    batch, seq, d = A_x.shape
    _, heads, sk, dh = A_k_cache.shape
    assert seq == 1 and batch < _ROWS and (heads, dh) == (_HEADS, _HEAD_DIM)
    assert len(_WO_HEADS) == 2 * _SLOTS and sum(_WO_HEADS) == heads and heads % _SLOTS == 0
    window = min(4096, max(256, sk // 4))
    assert window <= sk

    out = pl.pallas_call(
        _kernel,
        out_shape=jax.ShapeDtypeStruct((batch, d), A_x.dtype),
        in_specs=[pl.BlockSpec(memory_space=pl.ANY)] * 7,
        out_specs=pl.BlockSpec((batch, d), lambda: (0, 0)),
        scratch_shapes=[
            pltpu.VMEM((batch, d), A_x.dtype),
            pltpu.VMEM(A_wq.shape, A_wq.dtype),
            pltpu.VMEM(A_wo.shape, A_wo.dtype),
            pltpu.VMEM(B_w3.shape[::-1], B_w3.dtype),
            pltpu.VMEM(B_w4.shape, B_w4.dtype),
            pltpu.VMEM((_SLOTS, batch, window, dh), A_k_cache.dtype),
            pltpu.VMEM((_SLOTS, batch, window, dh), A_v_cache.dtype),
            pltpu.VMEM((_ROWS, heads * dh), jnp.float32),
        ],
        compiler_params=pltpu.CompilerParams(vmem_limit_bytes=48 * 2**20),
    )(A_x.reshape(batch, d), A_k_cache, A_v_cache, A_wq, A_wo, B_w3.T, B_w4)
    return out.reshape(batch, seq, d)
```

```python
import functools

import jax
import jax.numpy as jnp
from jax import lax
import jax.experimental.pallas as pl
import jax.experimental.pallas.tpu as pltpu

_HEADS = 32
_HEAD_DIM = 128
_EPS = 1e-5
_ROWS = 8
_SLOTS = 2
_KV_ROWS = 64
_KV_SPLIT = 4
_WO_HEADS = (20, 8, 3, 1)
_NT = (((1,), (1,)), ((), ()))


def _layernorm(x):
    m = jnp.mean(x, axis=-1, keepdims=True)
    c = x - m
    v = jnp.mean(c * c, axis=-1, keepdims=True)
    return c / jnp.sqrt(v + _EPS)


def _start(src, dst, idx, sem, priority):
    pltpu.make_async_copy(src.at[idx], dst.at[idx], sem).start(priority=priority)


def _wait_filled(buf, sem):
    pltpu.make_async_copy(buf, buf, sem).wait()


def _aligned(start, size):
    return pl.ds(pl.multiple_of(start, size), size)


def _compute(x_hbm, k_hbm, v_hbm, wq_hbm, wo_hbm, w3t_hbm, w4_hbm,
             x_buf, wq_buf, wo_buf, w3t_buf, w4_buf, kv_buf, o_buf, sems):
    batch, heads, sk, dh = k_hbm.shape
    window = kv_buf.shape[3]
    f32, mxu_dtype = jnp.float32, kv_buf.dtype
    wo_pieces = [(sum(_WO_HEADS[:i]), n, sems.at[_SLOTS + i]) for i, n in enumerate(_WO_HEADS)]

    def start_kv(h, slot):
        part = window // _KV_SPLIT

        @pl.loop(0, part // _KV_ROWS)
        def _(j):
            for s in range(_KV_SPLIT):
                r = s * part + j * _KV_ROWS
                for a, cache in enumerate((k_hbm, v_hbm)):
                    for priority, b in enumerate((pl.ds(0, 1), pl.ds(1, batch - 1))):
                        pltpu.make_async_copy(
                            cache.at[b, h, _aligned(sk - window + r, _KV_ROWS), :],
                            kv_buf.at[slot, a, b, _aligned(r, _KV_ROWS), :],
                            sems.at[slot],
                        ).start(priority=priority)

    def start_wo(h0, nh, sem):
        if nh % 4 == 0:
            @pl.loop(0, dh // 16)
            def _(j):
                r = _aligned(j * 16, 16)
                for h in range(h0, h0 + nh, 4):
                    _start(wo_hbm, wo_buf, (pl.ds(h, 1), r), sem, 0)
                    _start(wo_hbm, wo_buf, (pl.ds(h + 1, 3), r), sem, 1)
        else:
            @pl.loop(0, dh // 64)
            def _(j):
                for h in range(h0, h0 + nh):
                    _start(wo_hbm, wo_buf, (h, _aligned(j * 64, 16)), sem, 0)
                    _start(wo_hbm, wo_buf, (h, pl.ds(pl.multiple_of(j * 64 + 16, 16), 48)), sem, 1)

    def start_stream(sem):
        pltpu.make_async_copy(x_hbm, x_buf, sem).start()
        _, rows, cols = wq_hbm.shape

        @pl.loop(0, rows // 32)
        def _(j):
            for c in range(0, cols, 1024):
                for s in range(4):
                    r = _aligned(s * (rows // 4) + j * 8, 8)
                    _start(wq_hbm, wq_buf, (pl.ds(0, 1), r, pl.ds(c, 1024)), sem, 0)
                    _start(wq_hbm, wq_buf, (pl.ds(1, 3), r, pl.ds(c, 1024)), sem, 1)

        @pl.loop(0, w4_hbm.shape[1] // 16)
        def _(j):
            r = _aligned(j * 16, 16)
            _start(w3t_hbm, w3t_buf, (pl.ds(0, 1), r), sem, 0)
            _start(w3t_hbm, w3t_buf, (pl.ds(1, 1), r), sem, 1)
            _start(w4_hbm, w4_buf, (pl.ds(0, 2), r), sem, 1)

        start_kv(0, 0)
        for buf in (x_buf, wq_buf, w3t_buf, w4_buf):
            _wait_filled(buf, sem)

    pl.run_scoped(start_stream, pltpu.SemaphoreType.DMA)

    x = x_buf[...].astype(f32)
    xn = _layernorm(x)
    filler = jnp.zeros((_ROWS - batch, x.shape[1]), f32)

    def padded(a):
        return jnp.concatenate([a, filler], axis=0)

    xn_lhs = padded(xn).astype(mxu_dtype)
    mlp_lhs = padded(_layernorm(xn)).astype(mxu_dtype)
    acc = padded(x + xn)
    for i in range(w4_buf.shape[0]):
        hid = lax.dot_general(mlp_lhs, w3t_buf[i], _NT, preferred_element_type=f32)
        hid = jax.nn.gelu(hid, approximate=True).astype(mxu_dtype)
        acc = acc + jnp.dot(hid, w4_buf[i], preferred_element_type=f32)

    start_kv(1, 1)

    s_row = lax.broadcasted_iota(jnp.int32, (_ROWS, window), 0)
    o_row = lax.broadcasted_iota(jnp.int32, (_ROWS, dh), 0)

    @pl.loop(0, heads)
    def _(h):
        slot = lax.rem(h, _SLOTS)
        cols = _aligned(h * dh, dh)
        wq = wq_buf[:, :, cols].reshape(-1, dh)
        q = jnp.dot(xn_lhs, wq, preferred_element_type=f32).astype(mxu_dtype)

        _wait_filled(kv_buf.at[slot], sems.at[slot])
        s = lax.dot_general(q, kv_buf[slot, 0, 0], _NT, preferred_element_type=f32)
        for b in range(1, batch):
            s_b = lax.dot_general(q, kv_buf[slot, 0, b], _NT, preferred_element_type=f32)
            s = jnp.where(s_row == b, s_b, s)

        s = s * (dh ** -0.5)
        p = jnp.exp(s - jnp.max(s, axis=-1, keepdims=True))
        denom = jnp.sum(p, axis=-1, keepdims=True)
        p = p.astype(mxu_dtype)

        o = jnp.dot(p, kv_buf[slot, 1, 0], preferred_element_type=f32)
        for b in range(1, batch):
            o_b = jnp.dot(p, kv_buf[slot, 1, b], preferred_element_type=f32)
            o = jnp.where(o_row == b, o_b, o)
        o_buf[:, cols] = o / denom

        pl.when(h + _SLOTS < heads)(lambda: start_kv(h + _SLOTS, slot))
        pl.when(h + _SLOTS == heads)(lambda: start_wo(*wo_pieces[0]))

    for piece in wo_pieces[1:]:
        start_wo(*piece)

    for h0, nh, sem in wo_pieces:
        o = o_buf[:, pl.ds(h0 * dh, nh * dh)].astype(mxu_dtype)
        _wait_filled(wo_buf.at[pl.ds(h0, nh)], sem)
        wo = wo_buf[pl.ds(h0, nh)].reshape(nh * dh, -1)
        acc = acc + jnp.dot(o, wo, preferred_element_type=f32)
    return acc


def _kernel(x_hbm, k_hbm, v_hbm, wq_hbm, wo_hbm, w3t_hbm, w4_hbm, out_ref, *buffers):
    acc = pl.run_scoped(
        functools.partial(_compute, x_hbm, k_hbm, v_hbm, wq_hbm, wo_hbm, w3t_hbm, w4_hbm, *buffers),
        pltpu.SemaphoreType.DMA((_SLOTS + len(_WO_HEADS),)),
    )
    out_ref[...] = acc[:out_ref.shape[0]].astype(out_ref.dtype)


@jax.jit
def pallas_parallel_sum__sliding_block_cached__mixer_s_mlp__decode_kernel(
    A_x: jax.Array,
    A_k_cache: jax.Array,
    A_v_cache: jax.Array,
    A_wq: jax.Array,
    A_wo: jax.Array,
    B_x: jax.Array,
    B_w1: jax.Array,
    B_w2: jax.Array,
    B_w3: jax.Array,
    B_w4: jax.Array,
):
    batch, seq, d = A_x.shape
    _, heads, sk, dh = A_k_cache.shape
    ff = B_w4.shape[0]
    window = min(4096, max(256, sk // 4))
    assert seq == 1 and 1 < batch < _ROWS and (heads, dh) == (_HEADS, _HEAD_DIM)
    assert window <= sk and window % (_KV_SPLIT * _KV_ROWS) == 0 and sk % _KV_ROWS == 0
    assert d % 128 == 0 and ff % 32 == 0 and sum(_WO_HEADS) == heads

    x = A_x.reshape(batch, d)
    weights = (
        A_wq.reshape(4, d // 4, heads * dh),
        A_wo.reshape(heads, dh, d),
        B_w3.T.reshape(2, ff // 2, d),
        B_w4.reshape(2, ff // 2, d),
    )
    out = pl.pallas_call(
        _kernel,
        out_shape=jax.ShapeDtypeStruct((batch, d), A_x.dtype),
        in_specs=[pl.BlockSpec(memory_space=pl.ANY)] * 7,
        out_specs=pl.BlockSpec((batch, d), lambda: (0, 0)),
        scratch_shapes=[
            *(pltpu.VMEM(a.shape, a.dtype) for a in (x, *weights)),
            pltpu.VMEM((_SLOTS, 2, batch, window, dh), A_k_cache.dtype),
            pltpu.VMEM((_ROWS, heads * dh), jnp.float32),
        ],
        compiler_params=pltpu.CompilerParams(vmem_limit_bytes=48 * 2**20),
    )(x, A_k_cache, A_v_cache, *weights)
    return out.reshape(batch, seq, d)
```

```python
import functools

import jax
import jax.numpy as jnp
from jax import lax
import jax.experimental.pallas as pl
import jax.experimental.pallas.tpu as pltpu

_HEADS = 32
_HEAD_DIM = 128
_EPS = 1e-5
_GROUP = 16
_STEP = 8
_KV_ROWS = 64
_W_BLOCKS = 8
_WO_PIECES = ((0, 8, 0, 2), (0, 8, 2, 1), (0, 4, 3, 1), (4, 4, 3, 1))
_NT = (((1,), (1,)), ((), ()))


def _layernorm(x):
    m = jnp.mean(x, axis=-1, keepdims=True)
    c = x - m
    v = jnp.mean(c * c, axis=-1, keepdims=True)
    return c / jnp.sqrt(v + _EPS)


def _aligned(start, size):
    return pl.ds(pl.multiple_of(start, size), size)


def _start_split(src, dst, sem):
    for i in range(0, src.shape[0], 4):
        for priority, part in enumerate((pl.ds(i, 1), pl.ds(i + 1, 3))):
            pltpu.make_async_copy(src.at[part], dst.at[part], sem).start(priority=priority)


def _wait_filled(buf, sem):
    pltpu.make_async_copy(buf, buf, sem).wait()


def _compute(x_hbm, k_hbm, v_hbm, wq_hbm, wo_hbm, w3t_hbm, w4_hbm,
             x_buf, wq_buf, wo_buf, w3t_buf, w4_buf, k_buf, v_buf, q_buf, p_buf, o_buf,
             k_sem, v_sem, wo_sem):
    pairs, sk, dh = k_hbm.shape
    batch = x_hbm.shape[0]
    heads = pairs // batch
    window = k_buf.shape[2]
    groups, steps = pairs // _GROUP, _GROUP // _STEP
    f32, mxu_dtype = jnp.float32, k_buf.dtype

    def start_cache(cache, buf, sem, g, part, parts):
        n = window // _KV_ROWS // parts
        slot = lax.rem(g, 2)

        @pl.loop(part * n, (part + 1) * n)
        def _(j):
            _start_split(
                cache.at[_aligned(g * _GROUP, _GROUP), _aligned(sk - window + j * _KV_ROWS, _KV_ROWS)],
                buf.at[slot, :, _aligned(j * _KV_ROWS, _KV_ROWS)],
                sem.at[slot],
            )

    start_k = functools.partial(start_cache, k_hbm, k_buf, k_sem)
    start_v = functools.partial(start_cache, v_hbm, v_buf, v_sem)

    def start_wo(piece, part, parts):
        b0, nb, h0, nh = _WO_PIECES[piece]
        n = nh * dh // 16 // parts

        @pl.loop(part * n, (part + 1) * n)
        def _(j):
            idx = (pl.ds(b0, nb), _aligned(h0 * dh + j * 16, 16))
            _start_split(wo_hbm.at[idx], wo_buf.at[idx], wo_sem.at[piece])

    def fetch_weights(sem):
        pltpu.make_async_copy(x_hbm, x_buf, sem).start()

        @pl.loop(0, wq_hbm.shape[1] // 8)
        def _(j):
            for c in range(0, wq_hbm.shape[2], 1024):
                idx = (slice(None), _aligned(j * 8, 8), pl.ds(c, 1024))
                _start_split(wq_hbm.at[idx], wq_buf.at[idx], sem)

        @pl.loop(0, w4_hbm.shape[1] // 16)
        def _(j):
            rows = _aligned(j * 16, 16)
            for priority, src, dst, half in ((0, w3t_hbm, w3t_buf, pl.ds(0, 1)),
                                             (1, w3t_hbm, w3t_buf, pl.ds(1, 1)),
                                             (1, w4_hbm, w4_buf, pl.ds(0, 2))):
                pltpu.make_async_copy(
                    src.at[half, rows], dst.at[half, rows], sem).start(priority=priority)

        start_k(0, 0, 1)
        for buf in (x_buf, wq_buf, w3t_buf, w4_buf):
            _wait_filled(buf, sem)

    pl.run_scoped(fetch_weights, pltpu.SemaphoreType.DMA)

    x = x_buf[...].astype(f32)
    xn = _layernorm(x)
    mlp_in = _layernorm(xn).astype(mxu_dtype)
    acc = x + xn
    for i in range(w4_buf.shape[0]):
        hid = lax.dot_general(mlp_in, w3t_buf[i], _NT, preferred_element_type=f32)
        hid = jax.nn.gelu(hid, approximate=True).astype(mxu_dtype)
        acc = acc + jnp.dot(hid, w4_buf[i], preferred_element_type=f32)

    def head_rows(h):
        return pl.ds(h, batch, stride=heads)

    @pl.loop(0, heads)
    def _(h):
        start_v(0, h, heads)
        wq = wq_buf[:, :, _aligned(h * dh, dh)].reshape(-1, dh)
        q_buf[head_rows(h), :] = jnp.dot(xn.astype(mxu_dtype), wq, preferred_element_type=f32)

    def own_rows(product):
        out = product(0)
        row = lax.broadcasted_iota(jnp.int32, out.shape, 0)
        for i in range(1, _STEP):
            out = jnp.where(row == i, product(i), out)
        return out

    @pl.loop(0, groups)
    def _(g):
        slot = lax.rem(g, 2)

        def prefetch(start_next, wo_piece, t):
            pl.when(g + 1 < groups)(lambda: start_next(g + 1, t, steps))
            pl.when(g + 1 == groups)(lambda: start_wo(wo_piece, t, steps))

        _wait_filled(k_buf.at[slot], k_sem.at[slot])

        @pl.loop(0, steps)
        def _(t):
            q = q_buf[_aligned(g * _GROUP + t * _STEP, _STEP), :].astype(mxu_dtype)
            s = own_rows(lambda i: lax.dot_general(
                q, k_buf[slot, t * _STEP + i], _NT, preferred_element_type=f32))
            s = s * (dh ** -0.5)
            p = jnp.exp(s - jnp.max(s, axis=-1, keepdims=True))
            p_buf[t] = p / jnp.sum(p, axis=-1, keepdims=True)
            prefetch(start_k, 0, t)

        _wait_filled(v_buf.at[slot], v_sem.at[slot])

        @pl.loop(0, steps)
        def _(t):
            p = p_buf[t].astype(mxu_dtype)
            o_buf[_aligned(g * _GROUP + t * _STEP, _STEP), :] = own_rows(lambda i: jnp.dot(
                p, v_buf[slot, t * _STEP + i], preferred_element_type=f32))
            prefetch(start_v, 1, t)

    for piece in range(2, len(_WO_PIECES)):
        start_wo(piece, 0, 1)

    for piece, (b0, nb, h0, nh) in enumerate(_WO_PIECES):
        o = jnp.concatenate([
            o_buf[head_rows(b * (heads // _W_BLOCKS) + h), :]
            for b in range(b0, b0 + nb) for h in range(h0, h0 + nh)
        ], axis=1).astype(mxu_dtype)
        wo = wo_buf.at[pl.ds(b0, nb), pl.ds(h0 * dh, nh * dh)]
        _wait_filled(wo, wo_sem.at[piece])
        acc = acc + jnp.dot(o, wo[...].reshape(nb * nh * dh, -1), preferred_element_type=f32)
    return acc


def _kernel(x_hbm, k_hbm, v_hbm, wq_hbm, wo_hbm, w3t_hbm, w4_hbm, out_ref, *buffers):
    acc = pl.run_scoped(
        functools.partial(_compute, x_hbm, k_hbm, v_hbm, wq_hbm, wo_hbm, w3t_hbm, w4_hbm, *buffers),
        pltpu.SemaphoreType.DMA((2,)),
        pltpu.SemaphoreType.DMA((2,)),
        pltpu.SemaphoreType.DMA((len(_WO_PIECES),)),
    )
    out_ref[...] = acc.astype(out_ref.dtype)


@jax.jit
def pallas_parallel_sum__sliding_block_cached__mixer_s_mlp__decode_kernel(
    A_x: jax.Array,
    A_k_cache: jax.Array,
    A_v_cache: jax.Array,
    A_wq: jax.Array,
    A_wo: jax.Array,
    B_x: jax.Array,
    B_w1: jax.Array,
    B_w2: jax.Array,
    B_w3: jax.Array,
    B_w4: jax.Array,
):
    batch, seq, d = A_x.shape
    _, heads, sk, dh = A_k_cache.shape
    ff = B_w4.shape[0]
    window = min(4096, max(256, sk // 4))
    assert seq == 1 and (heads, dh) == (_HEADS, _HEAD_DIM)
    assert window <= sk and window % (heads * _KV_ROWS) == 0 and sk % _KV_ROWS == 0
    assert d % (16 * _W_BLOCKS) == 0 and ff % 32 == 0

    x = A_x.reshape(batch, d)
    caches = (A_k_cache.reshape(batch * heads, sk, dh), A_v_cache.reshape(batch * heads, sk, dh))
    weights = (
        A_wq.reshape(_W_BLOCKS, d // _W_BLOCKS, heads * dh),
        A_wo.reshape(_W_BLOCKS, heads * dh // _W_BLOCKS, d),
        B_w3.T.reshape(2, ff // 2, d),
        B_w4.reshape(2, ff // 2, d),
    )
    out = pl.pallas_call(
        _kernel,
        out_shape=jax.ShapeDtypeStruct((batch, d), A_x.dtype),
        in_specs=[pl.BlockSpec(memory_space=pl.ANY)] * 7,
        out_specs=pl.BlockSpec((batch, d), lambda: (0, 0)),
        scratch_shapes=[
            *(pltpu.VMEM(a.shape, a.dtype) for a in (x, *weights)),
            *(pltpu.VMEM((2, _GROUP, window, dh), a.dtype) for a in caches),
            pltpu.VMEM((batch * heads, dh), jnp.float32),
            pltpu.VMEM((_GROUP // _STEP, _STEP, window), jnp.float32),
            pltpu.VMEM((batch * heads, dh), jnp.float32),
        ],
        compiler_params=pltpu.CompilerParams(vmem_limit_bytes=64 * 2**20),
    )(x, *caches, *weights)
    return out.reshape(batch, seq, d)
```

```python
import functools

import jax
import jax.numpy as jnp
from jax import lax
import jax.experimental.pallas as pl
import jax.experimental.pallas.tpu as pltpu

_HEADS = 32
_HEAD_DIM = 128
_EPS = 1e-5
_GROUP = 16
_STEP = 8
_KV_ROWS = 64
_W_BLOCKS = 8
_WO_PIECES = ((0, 8, 0, 2), (0, 8, 2, 1), (0, 4, 3, 1), (4, 4, 3, 1))
_NT = (((1,), (1,)), ((), ()))


def _layernorm(x):
    m = jnp.mean(x, axis=-1, keepdims=True)
    c = x - m
    v = jnp.mean(c * c, axis=-1, keepdims=True)
    return c / jnp.sqrt(v + _EPS)


def _aligned(start, size):
    return pl.ds(pl.multiple_of(start, size), size)


def _start_split(src, dst, sem):
    for i in range(0, src.shape[0], 4):
        for priority, part in enumerate((pl.ds(i, 1), pl.ds(i + 1, 3))):
            pltpu.make_async_copy(src.at[part], dst.at[part], sem).start(priority=priority)


def _wait_filled(buf, sem):
    pltpu.make_async_copy(buf, buf, sem).wait()


def _compute(x_hbm, k_hbm, v_hbm, wq_hbm, wo_hbm, w3t_hbm, w4_hbm,
             x_buf, wq_buf, wo_buf, w3t_buf, w4_buf, k_buf, v_buf, q_buf, p_buf, o_buf,
             k_sem, v_sem, wo_sem):
    pairs, sk, dh = k_hbm.shape
    batch = x_hbm.shape[0]
    heads = pairs // batch
    window = k_buf.shape[2]
    groups, steps = pairs // _GROUP, _GROUP // _STEP
    f32, mxu_dtype = jnp.float32, k_buf.dtype

    def start_cache(cache, buf, sem, g, part, parts):
        n = window // _KV_ROWS // parts
        slot = lax.rem(g, 2)

        @pl.loop(part * n, (part + 1) * n)
        def _(j):
            _start_split(
                cache.at[_aligned(g * _GROUP, _GROUP), _aligned(sk - window + j * _KV_ROWS, _KV_ROWS)],
                buf.at[slot, :, _aligned(j * _KV_ROWS, _KV_ROWS)],
                sem.at[slot],
            )

    start_k = functools.partial(start_cache, k_hbm, k_buf, k_sem)
    start_v = functools.partial(start_cache, v_hbm, v_buf, v_sem)

    def start_wo(piece, part, parts):
        b0, nb, h0, nh = _WO_PIECES[piece]
        n = nh * dh // 16 // parts

        @pl.loop(part * n, (part + 1) * n)
        def _(j):
            idx = (pl.ds(b0, nb), _aligned(h0 * dh + j * 16, 16))
            _start_split(wo_hbm.at[idx], wo_buf.at[idx], wo_sem.at[piece])

    def fetch_weights(x_sem, wq_sem, w3_sem, w4_sem):
        pltpu.make_async_copy(x_hbm, x_buf, x_sem).start()

        @pl.loop(0, wq_hbm.shape[1] // 8)
        def _(j):
            for c in range(0, wq_hbm.shape[2], 1024):
                idx = (slice(None), _aligned(j * 8, 8), pl.ds(c, 1024))
                _start_split(wq_hbm.at[idx], wq_buf.at[idx], wq_sem)

        @pl.loop(0, w4_hbm.shape[1] // 16)
        def _(j):
            rows = _aligned(j * 16, 16)
            for priority, halves, src, dst, sem in (
                (0, pl.ds(0, 1), w3t_hbm, w3t_buf, w3_sem),
                (1, pl.ds(1, 1), w3t_hbm, w3t_buf, w3_sem),
                (1, pl.ds(0, 2), w4_hbm, w4_buf, w4_sem),
            ):
                pltpu.make_async_copy(
                    src.at[halves, rows], dst.at[halves, rows], sem).start(priority=priority)

        start_k(0, 0, 1)
        for buf, sem in ((x_buf, x_sem), (wq_buf, wq_sem), (w3t_buf, w3_sem), (w4_buf, w4_sem)):
            _wait_filled(buf, sem)

    pl.run_scoped(fetch_weights, *[pltpu.SemaphoreType.DMA] * 4)

    x = x_buf[...].astype(f32)
    xn = _layernorm(x)
    mlp_in = _layernorm(xn).astype(mxu_dtype)
    acc = x + xn
    for i in range(w4_buf.shape[0]):
        hid = lax.dot_general(mlp_in, w3t_buf[i], _NT, preferred_element_type=f32)
        hid = jax.nn.gelu(hid, approximate=True).astype(mxu_dtype)
        acc = acc + jnp.dot(hid, w4_buf[i], preferred_element_type=f32)

    def head_rows(h):
        return pl.ds(h, batch, stride=heads)

    @pl.loop(0, heads)
    def _(h):
        start_v(0, h, heads)
        wq = wq_buf[:, :, _aligned(h * dh, dh)].reshape(-1, dh)
        q_buf[head_rows(h), :] = jnp.dot(xn.astype(mxu_dtype), wq, preferred_element_type=f32)

    def own_rows(product):
        out = product(0)
        row = lax.broadcasted_iota(jnp.int32, out.shape, 0)
        for i in range(1, _STEP):
            out = jnp.where(row == i, product(i), out)
        return out

    @pl.loop(0, groups)
    def _(g):
        slot = lax.rem(g, 2)

        def prefetch(start_next, wo_piece, t):
            pl.when(g + 1 < groups)(lambda: start_next(g + 1, t, steps))
            pl.when(g + 1 == groups)(lambda: start_wo(wo_piece, t, steps))

        _wait_filled(k_buf.at[slot], k_sem.at[slot])

        @pl.loop(0, steps)
        def _(t):
            q = q_buf[_aligned(g * _GROUP + t * _STEP, _STEP), :].astype(mxu_dtype)
            s = own_rows(lambda i: lax.dot_general(
                q, k_buf[slot, t * _STEP + i], _NT, preferred_element_type=f32))
            s = s * (dh ** -0.5)
            p = jnp.exp(s - jnp.max(s, axis=-1, keepdims=True))
            p_buf[t] = p / jnp.sum(p, axis=-1, keepdims=True)
            prefetch(start_k, 0, t)

        _wait_filled(v_buf.at[slot], v_sem.at[slot])

        @pl.loop(0, steps)
        def _(t):
            p = p_buf[t].astype(mxu_dtype)
            o_buf[_aligned(g * _GROUP + t * _STEP, _STEP), :] = own_rows(lambda i: jnp.dot(
                p, v_buf[slot, t * _STEP + i], preferred_element_type=f32))
            prefetch(start_v, 1, t)

    for piece in range(2, len(_WO_PIECES)):
        start_wo(piece, 0, 1)

    for piece, (b0, nb, h0, nh) in enumerate(_WO_PIECES):
        o = jnp.concatenate([
            o_buf[head_rows(b * (heads // _W_BLOCKS) + h), :]
            for b in range(b0, b0 + nb) for h in range(h0, h0 + nh)
        ], axis=1).astype(mxu_dtype)
        wo = wo_buf.at[pl.ds(b0, nb), pl.ds(h0 * dh, nh * dh)]
        _wait_filled(wo, wo_sem.at[piece])
        acc = acc + jnp.dot(o, wo[...].reshape(nb * nh * dh, -1), preferred_element_type=f32)
    return acc


def _kernel(x_hbm, k_hbm, v_hbm, wq_hbm, wo_hbm, w3t_hbm, w4_hbm, out_ref, *buffers):
    acc = pl.run_scoped(
        functools.partial(_compute, x_hbm, k_hbm, v_hbm, wq_hbm, wo_hbm, w3t_hbm, w4_hbm, *buffers),
        pltpu.SemaphoreType.DMA((2,)),
        pltpu.SemaphoreType.DMA((2,)),
        pltpu.SemaphoreType.DMA((len(_WO_PIECES),)),
    )
    out_ref[...] = acc.astype(out_ref.dtype)


@jax.jit
def pallas_parallel_sum__sliding_block_cached__mixer_s_mlp__decode_kernel(
    A_x: jax.Array,
    A_k_cache: jax.Array,
    A_v_cache: jax.Array,
    A_wq: jax.Array,
    A_wo: jax.Array,
    B_x: jax.Array,
    B_w1: jax.Array,
    B_w2: jax.Array,
    B_w3: jax.Array,
    B_w4: jax.Array,
):
    batch, seq, d = A_x.shape
    _, heads, sk, dh = A_k_cache.shape
    ff = B_w4.shape[0]
    window = min(4096, max(256, sk // 4))
    assert seq == 1 and (heads, dh) == (_HEADS, _HEAD_DIM)
    assert window <= sk and window % (heads * _KV_ROWS) == 0 and sk % _KV_ROWS == 0
    assert d % (16 * _W_BLOCKS) == 0 and ff % 32 == 0

    x = A_x.reshape(batch, d)
    caches = (A_k_cache.reshape(batch * heads, sk, dh), A_v_cache.reshape(batch * heads, sk, dh))
    weights = (
        A_wq.reshape(_W_BLOCKS, d // _W_BLOCKS, heads * dh),
        A_wo.reshape(_W_BLOCKS, heads * dh // _W_BLOCKS, d),
        B_w3.T.reshape(2, ff // 2, d),
        B_w4.reshape(2, ff // 2, d),
    )
    out = pl.pallas_call(
        _kernel,
        out_shape=jax.ShapeDtypeStruct((batch, d), A_x.dtype),
        in_specs=[pl.BlockSpec(memory_space=pl.ANY)] * 7,
        out_specs=pl.BlockSpec((batch, d), lambda: (0, 0)),
        scratch_shapes=[
            *(pltpu.VMEM(a.shape, a.dtype) for a in (x, *weights)),
            *(pltpu.VMEM((2, _GROUP, window, dh), a.dtype) for a in caches),
            pltpu.VMEM((batch * heads, dh), jnp.float32),
            pltpu.VMEM((_GROUP // _STEP, _STEP, window), jnp.float32),
            pltpu.VMEM((batch * heads, dh), jnp.float32),
        ],
        compiler_params=pltpu.CompilerParams(vmem_limit_bytes=64 * 2**20),
    )(x, *caches, *weights)
    return out.reshape(batch, seq, d)
```
